```python
import jax
import jax.numpy as jnp

def _softmax(x, axis=-1):
    return jax.nn.softmax(x, axis=axis)

def _gelu(x):
    return jax.nn.gelu(x, approximate=True)

def _silu(x):
    return jax.nn.silu(x)

def _sigmoid(x):
    return jax.nn.sigmoid(x)

def _layernorm(x, axis=-1, eps=1e-05):
    m = jnp.mean(x, axis=axis, keepdims=True)
    v = jnp.var(x, axis=axis, keepdims=True)
    return (x - m) / jnp.sqrt(v + eps)

def _scatter_add(tgt, idx, src, axis=0):
    return tgt.at[idx].add(src)

def _segment_sum(src, seg, n):
    return jax.ops.segment_sum(src, seg, n)

class _Rng:

    def __init__(self, key):
        self._k = key

    def _next(self):
        self._k, sub = jax.random.split(self._k)
        return sub

    def normal(self, shape):
        return jax.random.normal(self._next(), shape, dtype=jnp.bfloat16)

    def randint(self, lo, hi, shape):
        return jax.random.randint(self._next(), shape, lo, hi, dtype=jnp.int32)

    def uniform(self, shape, lo=0.0, hi=1.0):
        return jax.random.uniform(self._next(), shape, jnp.bfloat16, lo, hi)

    def permutation(self, n):
        return jax.random.permutation(self._next(), n)
kernel_name = 'adaLN_cond__memory_aug_recurrent_mem_tr__dense_activation_gelu__prompt'

def setup_inputs():
    _rng = _Rng(jax.random.key(int.from_bytes(__import__("os").urandom(4), "little")))
    _w = lambda a: (lambda t: t.astype(jnp.bfloat16) if jnp.issubdtype(t.dtype, jnp.floating) else t)(jnp.asarray(a))

    def _A_setup():
        B, S, Dm = (1, 2048, 1024)
        H, Dh = (32, 128)
        M, seg = (8, 32)
        seg = min(seg, S)
        S = S // seg * seg
        return {'x': _w((lambda *s: _rng.normal(s) * 0.05)(B, S, Dm)), 'mem0': _w((lambda *s: _rng.normal(s) * 0.05)(B, M, Dm)), 'Wq': _w((lambda *s: _rng.normal(s) * 0.05)(Dm, H, Dh) * Dm ** (-0.5)), 'Wk': _w((lambda *s: _rng.normal(s) * 0.05)(Dm, H, Dh) * Dm ** (-0.5)), 'Wv': _w((lambda *s: _rng.normal(s) * 0.05)(Dm, H, Dh) * Dm ** (-0.5)), 'Wo': _w((lambda *s: _rng.normal(s) * 0.05)(H, Dh, Dm) * (H * Dh) ** (-0.5)), 'seg_len': seg}
    _A_in = _A_setup()

    def _B_setup():
        B, S, D, F = (1, 2048, 1024, 3584)
        return {'x': _w((lambda *s: _rng.normal(s) * 0.05)(B, S, D)), 'w1': _w((lambda *s: _rng.normal(s) * 0.05)(D, F) * D ** (-0.5)), 'b1': _w((lambda *s: _rng.normal(s) * 0.05)(F) * 0.01), 'w2': _w((lambda *s: _rng.normal(s) * 0.05)(F, D) * F ** (-0.5)), 'b2': _w((lambda *s: _rng.normal(s) * 0.05)(D) * 0.01)}
    _B_in = _B_setup()
    return {'A_x': _A_in['x'], 'A_mem0': _A_in['mem0'], 'A_Wq': _A_in['Wq'], 'A_Wk': _A_in['Wk'], 'A_Wv': _A_in['Wv'], 'A_Wo': _A_in['Wo'], 'A_seg_len': _A_in['seg_len'], 'B_x': _B_in['x'], 'B_w1': _B_in['w1'], 'B_b1': _B_in['b1'], 'B_w2': _B_in['w2'], 'B_b2': _B_in['b2'], 'c': _w((lambda *s: _rng.normal(s) * 0.05)(1, 1024)), 'w_mod': _w((lambda *s: _rng.normal(s) * 0.05)(1024, 6 * 1024) * 1024 ** (-0.5))}

def reference(A_x, A_mem0, A_Wq, A_Wk, A_Wv, A_Wo, A_seg_len, B_x, B_w1, B_b1, B_w2, B_b2, c, w_mod):

    def _A_ref(x, mem0, Wq, Wk, Wv, Wo, seg_len):
        B, S, Dm = x.shape
        H, Dh = (Wq.shape[1], Wq.shape[2])
        M = mem0.shape[1]
        scale = Dh ** (-0.5)
        n_seg = S // seg_len
        L = M + seg_len
        idx = jnp.arange(L)
        mask = (idx[:, None] < M) | (idx[:, None] >= idx[None, :])
        mem = mem0
        outs = []
        for s in range(n_seg):
            xs = x[:, s * seg_len:(s + 1) * seg_len, :].copy()
            h = jnp.concatenate([mem, xs], axis=1)
            q = jnp.einsum('btd,dhe->bhte', h, Wq)
            k = jnp.einsum('btd,dhe->bhte', h, Wk)
            v = jnp.einsum('btd,dhe->bhte', h, Wv)
            scores = jnp.einsum('bhqe,bhke->bhqk', q, k) * scale
            scores = jnp.where(mask[None, None], scores, -1000000000.0)
            p = _softmax(scores, axis=-1)
            o = jnp.einsum('bhqk,bhke->bhqe', p, v)
            o = jnp.einsum('bhte,hed->btd', o, Wo)
            mem = o[:, :M, :].copy()
            outs.append(o[:, M:, :])
        return jnp.concatenate(outs, axis=1)

    def _B_ref(x, w1, b1, w2, b2):
        h = jnp.einsum('bsd,df->bsf', x, w1) + b1
        h = _gelu(h)
        return jnp.einsum('bsf,fd->bsd', h, w2) + b2
    x = A_x
    mod = (_silu(c) @ w_mod).reshape(c.shape[0], 6, 1, -1)
    sa, ca, ga, sb, cb, gb = (mod[:, 0].copy(), mod[:, 1].copy(), mod[:, 2].copy(), mod[:, 3].copy(), mod[:, 4].copy(), mod[:, 5].copy())
    h = _layernorm(x, axis=-1) * (1 + ca) + sa
    x = x + ga * _A_ref(h, A_mem0, A_Wq, A_Wk, A_Wv, A_Wo, A_seg_len)
    h = _layernorm(x, axis=-1) * (1 + cb) + sb
    x = x + gb * _B_ref(h, B_w1, B_b1, B_w2, B_b2)
    return x
```

```python
import functools
import numpy as np
import jax
import jax.numpy as jnp
import jax.experimental.pallas as pl
import jax.experimental.pallas.tpu as pltpu

F32 = jnp.float32
BF16 = jnp.bfloat16
U32 = jnp.uint32
NEG = -1000000000.0


def _ln(x, eps=1e-5):
    m = jnp.mean(x, axis=-1, keepdims=True)
    xc = x - m
    v = jnp.mean(xc * xc, axis=-1, keepdims=True)
    return xc * jax.lax.rsqrt(v + eps)


def _gelu(x):
    c = float(np.sqrt(2.0 / np.pi))
    return 0.5 * x * (1.0 + jnp.tanh(c * (x + 0.044715 * (x * x * x))))


def _nt(a, b):
    return jax.lax.dot_general(a, b, (((1,), (1,)), ((), ())), preferred_element_type=F32)


def _mm(a, b):
    return jnp.dot(a, b, preferred_element_type=F32)


def _kernel(x_hbm, mem0_ref, wq_hbm, wk_hbm, wv_hbm, wo_hbm, w1_hbm, b1_ref, w2_hbm, b2_ref, c_ref, wmod_hbm,
            out_hbm,
            x_v, wqkv_v, wo_v, w1_v, w2_v, wmod_v, stage_v, ox_v, x1_v, out_v, sems, wsems, osems,
            *, S, D, H, Dh, Fd, M, seg):
    HD = H * Dh
    NP = S // (2 * seg)
    scale = float(Dh) ** -0.5
    DC = 128
    NCH = D // DC

    cp_mod = pltpu.make_async_copy(wmod_hbm.bitcast(U32), wmod_v, sems.at[0])
    cp_x = pltpu.make_async_copy(x_hbm, x_v, sems.at[1])
    cp_wo = pltpu.make_async_copy(wo_hbm.bitcast(U32), wo_v, sems.at[2])
    cp_w1 = pltpu.make_async_copy(w1_hbm.bitcast(U32), w1_v, sems.at[3])
    cp_w2 = pltpu.make_async_copy(w2_hbm.bitcast(U32), w2_v, sems.at[4])
    cp_mod.start()
    cp_x.start()
    wcps = []
    for mi, w_hbm in enumerate((wq_hbm, wk_hbm, wv_hbm)):
        for ci in range(NCH):
            k = mi * NCH + ci
            cp = pltpu.make_async_copy(w_hbm.at[pl.ds(ci * DC, DC)], stage_v.at[k], wsems.at[k])
            cp.start()
            wcps.append(cp)
    cp_wo.start()

    cp_mod.wait()
    cc = c_ref[...].astype(F32)
    sc = (cc * jax.nn.sigmoid(cc)).astype(BF16)
    sc = jnp.broadcast_to(sc, (16, D))
    mod = _mm(sc, pltpu.bitcast(wmod_v[...], BF16))[0:1, :]
    sa, ca, ga, sb, cb, gb = [mod[:, i * D:(i + 1) * D] for i in range(6)]

    for mi in range(3):
        for ci in range(NCH):
            k = mi * NCH + ci
            wcps[k].wait()
            w = pltpu.bitcast(stage_v[k].reshape(DC, HD), U32)
            for g in range(H // 4):
                wqkv_v[ci * DC // 2:(ci + 1) * DC // 2, g * 1536 + mi * 512: g * 1536 + (mi + 1) * 512] = w[:, g * 512:(g + 1) * 512]
    cp_w1.start()
    cp_w2.start()
    cp_x.wait()
    cp_wo.wait()

    ox_v[...] = jnp.zeros(ox_v.shape, F32)

    LA = 48
    r = jax.lax.broadcasted_iota(jnp.int32, (LA, LA), 0)
    cidx = jax.lax.broadcasted_iota(jnp.int32, (LA, LA), 1)
    L = M + seg
    maskA = (cidx < L) & ((r < M) | (r >= cidx))
    def posB(i):
        return jnp.where(i < M, i, jnp.where(i < 32, i + 8, jnp.where(i < 40, i - 24, 1000)))
    pr, pc = posB(r), posB(cidx)
    maskB = (cidx < L) & ((pr < M) | (pr >= pc))

    def attn(q, k, v, mask):
        s = _nt(q.astype(BF16), k.astype(BF16)) * scale
        s = jnp.where(mask, s, NEG)
        m = jnp.max(s, axis=-1, keepdims=True)
        e = jnp.exp(s - m)
        p = e / jnp.sum(e, axis=-1, keepdims=True)
        return _mm(p.astype(BF16), v.astype(BF16))

    NG = H // 4

    def scores(q, k, mask):
        s = _nt(q.astype(BF16), k.astype(BF16)) * scale
        s = jnp.where(mask, s, NEG)
        m = jnp.max(s, axis=-1, keepdims=True)
        e = jnp.exp(s - m)
        return (e / jnp.sum(e, axis=-1, keepdims=True)).astype(BF16)

    def step(lhs, oxl, mask, extra, nxkeep):
        qkv = {}
        ps = {}
        y = None
        keep = []
        ox = []
        z8 = jnp.zeros((8, Dh), F32)
        for t in range(NG + 2):
            if t < NG:
                qkv[t] = _mm(lhs, pltpu.bitcast(wqkv_v[:, t * 1536:(t + 1) * 1536], BF16))
            if 0 <= t - 1 < NG:
                g = t - 1
                for j in range(4):
                    h = g * 4 + j
                    q = qkv[g][:, j * 128:(j + 1) * 128]
                    k = qkv[g][:, 512 + j * 128:512 + (j + 1) * 128]
                    v = qkv[g][:, 1024 + j * 128:1024 + (j + 1) * 128]
                    if extra is not None:
                        q = jnp.concatenate([q, extra[h][0], z8], axis=0)
                        k = jnp.concatenate([k, extra[h][1], z8], axis=0)
                        v = jnp.concatenate([v, extra[h][2], z8], axis=0)
                    else:
                        keep.append((q[40:48], k[40:48], v[40:48]))
                    ps[h] = (scores(q, k, mask), v.astype(BF16))
            if 0 <= t - 2 < NG:
                g = t - 2
                os_ = []
                for j in range(4):
                    h = g * 4 + j
                    o = _mm(ps[h][0], ps[h][1])
                    os_.append(o)
                oc = jnp.concatenate(os_, axis=1)
                ox.append(oc[8:40])
                lo = jnp.concatenate([oc[0:8], oxl[:, g * 512:(g + 1) * 512]], axis=0).astype(BF16)
                yy = _mm(lo, pltpu.bitcast(wo_v[g * 256:(g + 1) * 256, :], BF16))
                y = yy if y is None else y + yy
        return y, ox, keep

    def pair(p, mem):
        r0 = pl.multiple_of(p * 64, 64)
        xr = x_v[pl.ds(r0, 64), :].astype(F32)
        hx = _ln(xr) * (1.0 + ca) + sa
        lhsA = jnp.concatenate([mem, hx[0:40]], axis=0).astype(BF16)
        ya, oxa, keep = step(lhsA, ox_v[0:40, :], maskA, None, None)
        lhsB = jnp.concatenate([ya[0:8], hx[40:64]], axis=0).astype(BF16)
        yb, oxb, _ = step(lhsB, ox_v[40:64, :], maskB, keep, None)
        oxb = [jnp.concatenate([o[24:32], o[0:24]], axis=0) for o in oxb]
        rp = pl.multiple_of(jnp.maximum(p - 1, 0) * 64, 64)
        xp = x_v[pl.ds(rp, 64), :].astype(F32)
        att = jnp.concatenate([ya[8:48], yb[8:32]], axis=0)
        x1_v[pl.ds(rp, 64), :] = xp + ga * att
        ox_v[0:32, :] = jnp.concatenate(oxa, axis=1)
        ox_v[32:64, :] = jnp.concatenate(oxb, axis=1)
        return yb[0:8]

    mem = jax.lax.fori_loop(0, NP, pair, mem0_ref[...].astype(F32))
    rp = (NP - 1) * 64
    att = _mm(ox_v[...].astype(BF16), pltpu.bitcast(wo_v[...], BF16))
    x1_v[pl.ds(rp, 64), :] = x_v[pl.ds(rp, 64), :].astype(F32) + ga * att

    cp_w1.wait()
    cp_w2.wait()
    b1 = b1_ref[...].astype(F32)
    b2 = b2_ref[...].astype(F32)
    RB = 256
    NB = S // RB

    def out_cp(i, slot):
        return pltpu.make_async_copy(out_v.at[slot], out_hbm.at[pl.ds(pl.multiple_of(i * RB, RB), RB)], osems.at[slot])

    def ffn(i, _):
        slot = i % 2
        r0 = pl.multiple_of(i * RB, RB)
        x1 = x1_v[pl.ds(r0, RB), :]
        h2 = (_ln(x1) * (1.0 + cb) + sb).astype(BF16)
        a = _gelu(_mm(h2, pltpu.bitcast(w1_v[...], BF16)) + b1).astype(BF16)
        y = _mm(a, pltpu.bitcast(w2_v[...], BF16)) + b2

        @pl.when(i >= 2)
        def _():
            out_cp(i - 2, slot).wait()
        out_v[slot] = (x1 + gb * y).astype(BF16)
        out_cp(i, slot).start()
        return 0

    jax.lax.fori_loop(0, NB, ffn, 0)
    out_cp(NB - 2, (NB - 2) % 2).wait()
    out_cp(NB - 1, (NB - 1) % 2).wait()


@functools.partial(jax.jit, static_argnames=("A_seg_len",))
def pallas_adaLN_cond__memory_aug_recurrent_mem_tr__dense_activation_gelu__prompt_kernel(
        A_x, A_mem0, A_Wq, A_Wk, A_Wv, A_Wo, A_seg_len, B_x, B_w1, B_b1, B_w2, B_b2, c, w_mod):
    B, S, D = A_x.shape
    H, Dh = A_Wq.shape[1], A_Wq.shape[2]
    M = A_mem0.shape[1]
    Fd = B_w1.shape[1]
    seg = int(A_seg_len)
    assert B == 1 and M == 8 and seg == 32 and Dh == 128
    HD = H * Dh
    anyspec = pl.BlockSpec(memory_space=pl.ANY)
    vm = pl.BlockSpec(memory_space=pltpu.VMEM)
    out = pl.pallas_call(
        functools.partial(_kernel, S=S, D=D, H=H, Dh=Dh, Fd=Fd, M=M, seg=seg),
        out_shape=jax.ShapeDtypeStruct((S, D), BF16),
        in_specs=[anyspec, vm, anyspec, anyspec, anyspec, anyspec, anyspec, vm, anyspec, vm, vm, anyspec],
        out_specs=anyspec,
        scratch_shapes=[
            pltpu.VMEM((S, D), BF16),
            pltpu.VMEM((D // 2, 3 * HD), U32),
            pltpu.VMEM((HD // 2, D), U32),
            pltpu.VMEM((D // 2, Fd), U32),
            pltpu.VMEM((Fd // 2, D), U32),
            pltpu.VMEM((D // 2, 6 * D), U32),
            pltpu.VMEM((3 * D // 128, 128, H, Dh), BF16),
            pltpu.VMEM((64, HD), F32),
            pltpu.VMEM((S, D), F32),
            pltpu.VMEM((2, 256, D), BF16),
            pltpu.SemaphoreType.DMA((5,)),
            pltpu.SemaphoreType.DMA((3 * D // 128,)),
            pltpu.SemaphoreType.DMA((2,)),
        ],
        compiler_params=pltpu.CompilerParams(vmem_limit_bytes=120 * 1024 * 1024),
    )(A_x.reshape(S, D), A_mem0.reshape(M, D), A_Wq, A_Wk, A_Wv, A_Wo.reshape(HD, D), B_w1, B_b1.reshape(1, Fd),
      B_w2, B_b2.reshape(1, D), c, w_mod)
    return out.reshape(B, S, D)
```

```python
import functools
import numpy as np
import jax
import jax.numpy as jnp
import jax.experimental.pallas as pl
import jax.experimental.pallas.tpu as pltpu

F32 = jnp.float32
BF16 = jnp.bfloat16
U32 = jnp.uint32
NEG = -1000000000.0


def _ln(x, eps=1e-5):
    m = jnp.mean(x, axis=-1, keepdims=True)
    xc = x - m
    v = jnp.mean(xc * xc, axis=-1, keepdims=True)
    return xc * jax.lax.rsqrt(v + eps)


def _gelu(x):
    c = float(np.sqrt(2.0 / np.pi))
    return 0.5 * x * (1.0 + jnp.tanh(c * (x + 0.044715 * (x * x * x))))


def _nt(a, b):
    return jax.lax.dot_general(a, b, (((1,), (1,)), ((), ())), preferred_element_type=F32)


def _mm(a, b):
    return jnp.dot(a, b, preferred_element_type=F32)


def _kernel(x_hbm, mem0_ref, wq_hbm, wk_hbm, wv_hbm, wo_hbm, w1_hbm, b1_ref, w2_hbm, b2_ref, c_ref, wmod_hbm,
            out_hbm,
            x_v, wqkv_v, wo_v, w1_v, w2_v, wmod_v, stage_v, ox_v, x1_v, outf_v, sems, wsems, osems,
            *, S, D, H, Dh, Fd, M, seg):
    HD = H * Dh
    NP = S // (2 * seg)
    scale = float(Dh) ** -0.5
    NST = stage_v.shape[0]
    NCH = 3 * (H // 8)
    XF = 128

    def wchunk_cp(k):
        cblk, mi = divmod(k, 3)
        w_hbm = (wq_hbm, wk_hbm, wv_hbm)[mi]
        return pltpu.make_async_copy(w_hbm.at[:, pl.ds(cblk * 8, 8), :], stage_v.at[k % NST], wsems.at[k])

    wmod32 = wmod_hbm.bitcast(U32)
    cp_modA = pltpu.make_async_copy(wmod32.at[:, pl.ds(0, 2 * D)], wmod_v.at[:, pl.ds(0, 2 * D)], sems.at[0])
    cp_modB = pltpu.make_async_copy(wmod32.at[:, pl.ds(2 * D, 4 * D)], wmod_v.at[:, pl.ds(2 * D, 4 * D)], sems.at[5])
    cp_x0 = pltpu.make_async_copy(x_hbm.at[pl.ds(0, XF)], x_v.at[pl.ds(0, XF)], sems.at[1])
    cp_x1 = pltpu.make_async_copy(x_hbm.at[pl.ds(XF, S - XF)], x_v.at[pl.ds(XF, S - XF)], sems.at[6])
    cp_wo = pltpu.make_async_copy(wo_hbm.bitcast(U32), wo_v, sems.at[2])
    cp_w1 = pltpu.make_async_copy(w1_hbm.bitcast(U32), w1_v, sems.at[3])
    cp_w2 = pltpu.make_async_copy(w2_hbm.bitcast(U32), w2_v, sems.at[4])

    cp_modA.start()
    cp_x0.start()
    for k in range(NST - 1):
        wchunk_cp(k).start()

    cc = c_ref[...].astype(F32)
    sc = (cc * jax.nn.sigmoid(cc)).astype(BF16)
    sc = jnp.broadcast_to(sc, (16, D))
    cp_modA.wait()
    modA = _mm(sc, pltpu.bitcast(wmod_v[:, 0:2 * D], BF16))[0:1, :]
    sa, ca = modA[:, 0:D], modA[:, D:2 * D]

    for k in range(NCH):
        cblk, mi = divmod(k, 3)
        wchunk_cp(k).wait()
        if k + NST - 1 < NCH:
            wchunk_cp(k + NST - 1).start()
        elif k + NST - 1 == NCH:
            cp_wo.start()
        elif k + NST - 1 == NCH + 1:
            cp_x1.start()
        w = pltpu.bitcast(stage_v[k % NST].reshape(D, 8 * Dh), U32)
        for gg in range(2):
            g = cblk * 2 + gg
            wqkv_v[:, g * 1536 + mi * 512: g * 1536 + (mi + 1) * 512] = w[:, gg * 512:(gg + 1) * 512]
    cp_x0.wait()
    cp_wo.wait()
    cp_modB.start()
    cp_w1.start()
    cp_w2.start()

    ox_v[...] = jnp.zeros(ox_v.shape, F32)

    LA = 48
    r = jax.lax.broadcasted_iota(jnp.int32, (LA, LA), 0)
    cidx = jax.lax.broadcasted_iota(jnp.int32, (LA, LA), 1)
    L = M + seg
    maskA = (cidx < L) & ((r < M) | (r >= cidx))
    def posB(i):
        return jnp.where(i < M, i, jnp.where(i < 32, i + 8, jnp.where(i < 40, i - 24, 1000)))
    pr, pc = posB(r), posB(cidx)
    maskB = (cidx < L) & ((pr < M) | (pr >= pc))

    def attn(q, k, v, mask):
        s = _nt(q.astype(BF16), k.astype(BF16)) * scale
        s = jnp.where(mask, s, NEG)
        m = jnp.max(s, axis=-1, keepdims=True)
        e = jnp.exp(s - m)
        p = e / jnp.sum(e, axis=-1, keepdims=True)
        return _mm(p.astype(BF16), v.astype(BF16))

    NG = H // 4

    def scores(q, k, mask):
        s = _nt(q.astype(BF16), k.astype(BF16)) * scale
        s = jnp.where(mask, s, NEG)
        m = jnp.max(s, axis=-1, keepdims=True)
        e = jnp.exp(s - m)
        return (e / jnp.sum(e, axis=-1, keepdims=True)).astype(BF16)

    def step(lhs, oxl, mask, extra, fill):
        qkv = {}
        ps = {}
        y = None
        keep = []
        ox = []
        z8 = jnp.zeros((8, Dh), F32)
        for t in range(NG + 2):
            if t < NG:
                qkv[t] = _mm(lhs, pltpu.bitcast(wqkv_v[:, t * 1536:(t + 1) * 1536], BF16))
            if 0 <= t - 1 < NG:
                g = t - 1
                for j in range(4):
                    h = g * 4 + j
                    q = qkv[g][:, j * 128:(j + 1) * 128]
                    k = qkv[g][:, 512 + j * 128:512 + (j + 1) * 128]
                    v = qkv[g][:, 1024 + j * 128:1024 + (j + 1) * 128]
                    if extra is not None:
                        q = jnp.concatenate([q, extra[h][0], z8], axis=0)
                        k = jnp.concatenate([k, extra[h][1], z8], axis=0)
                        v = jnp.concatenate([v, extra[h][2], z8], axis=0)
                    else:
                        keep.append((q[40:48], k[40:48], v[40:48]))
                    ps[h] = (scores(q, k, mask), v.astype(BF16))
                if g >= NG - 2 or g == 2:
                    fill()
            if 0 <= t - 2 < NG:
                g = t - 2
                os_ = []
                for j in range(4):
                    h = g * 4 + j
                    o = _mm(ps[h][0], ps[h][1])
                    os_.append(o)
                oc = jnp.concatenate(os_, axis=1)
                if g == NG - 1:
                    fill()
                ox.append(oc[8:40])
                lo = jnp.concatenate([oc[0:8], oxl[:, g * 512:(g + 1) * 512]], axis=0).astype(BF16)
                yy = _mm(lo, pltpu.bitcast(wo_v[g * 256:(g + 1) * 256, :], BF16))
                y = yy if y is None else y + yy
                if g >= NG - 2:
                    fill()
        fill()
        return y, ox, keep

    def pair(p, mem, with_ffn):
        @pl.when(p == XF // 64)
        def _():
            cp_x1.wait()

        r0 = pl.multiple_of(p * 64, 64)
        xr = x_v[pl.ds(r0, 64), :].astype(F32)
        hx = _ln(xr) * (1.0 + ca) + sa
        lhsA = jnp.concatenate([mem, hx[0:40]], axis=0).astype(BF16)
        st = {"i": 0, "a": {}, "y": None}
        if with_ffn:
            rf = pl.multiple_of((p - 2) * 64, 64)
            x1f = x_v[pl.ds(rf, 64), :].astype(F32) + ga * x1_v[pl.ds(rf, 64), :]
            h2 = (_ln(x1f) * (1.0 + cb) + sb).astype(BF16)

        def fill():
            if not with_ffn:
                return
            i = st["i"]
            st["i"] = i + 1
            if i < 7:
                st["a"][i] = _gelu(_mm(h2, pltpu.bitcast(w1_v[:, i * 512:(i + 1) * 512], BF16)) + b1[:, i * 512:(i + 1) * 512]).astype(BF16)
            else:
                j = i - 7
                yy = _mm(st["a"][j], pltpu.bitcast(w2_v[j * 256:(j + 1) * 256, :], BF16))
                st["y"] = yy if st["y"] is None else st["y"] + yy

        ya, oxa, keep = step(lhsA, ox_v[0:40, :], maskA, None, fill)
        lhsB = jnp.concatenate([ya[0:8], hx[40:64]], axis=0).astype(BF16)
        yb, oxb, _ = step(lhsB, ox_v[40:64, :], maskB, keep, fill)
        oxb = [jnp.concatenate([o[24:32], o[0:24]], axis=0) for o in oxb]
        rp = pl.multiple_of(jnp.maximum(p - 1, 0) * 64, 64)
        att = jnp.concatenate([ya[8:48], yb[8:32]], axis=0)
        x1_v[pl.ds(rp, 64), :] = att
        ox_v[0:32, :] = jnp.concatenate(oxa, axis=1)
        ox_v[32:64, :] = jnp.concatenate(oxb, axis=1)
        if with_ffn:
            assert st["i"] == 14, st["i"]
            outf_v[pl.ds(rf, 64), :] = (x1f + gb * (st["y"] + b2)).astype(BF16)
        return yb[0:8]

    mem = jax.lax.fori_loop(0, 2, lambda p, m: pair(p, m, False), mem0_ref[...].astype(F32))
    cp_modB.wait()
    modB = _mm(sc, pltpu.bitcast(wmod_v[:, 2 * D:6 * D], BF16))[0:1, :]
    ga, sb, cb, gb = [modB[:, i * D:(i + 1) * D] for i in range(4)]
    cp_w1.wait()
    cp_w2.wait()
    b1 = b1_ref[...].astype(F32).reshape(1, Fd)
    b2 = b2_ref[...].astype(F32).reshape(1, D)
    with jax.named_scope('mainloop'):
        mem = jax.lax.fori_loop(2, NP, lambda p, m: pair(p, m, True), mem)
    HALF = S // 2
    oc0 = pltpu.make_async_copy(outf_v.at[pl.ds(0, S - 128)], out_hbm.at[pl.ds(0, S - 128)], osems.at[0])
    oc0.start()
    rp = (NP - 1) * 64
    x1_v[pl.ds(rp, 64), :] = _mm(ox_v[...].astype(BF16), pltpu.bitcast(wo_v[...], BF16))
    r0 = S - 128
    x1 = x_v[pl.ds(r0, 128), :].astype(F32) + ga * x1_v[pl.ds(r0, 128), :]
    h2 = (_ln(x1) * (1.0 + cb) + sb).astype(BF16)
    a = _gelu(_mm(h2, pltpu.bitcast(w1_v[...], BF16)) + b1).astype(BF16)
    y = _mm(a, pltpu.bitcast(w2_v[...], BF16)) + b2
    outf_v[pl.ds(r0, 128), :] = (x1 + gb * y).astype(BF16)
    oc1 = pltpu.make_async_copy(outf_v.at[pl.ds(r0, 128)], out_hbm.at[pl.ds(r0, 128)], osems.at[1])
    oc1.start()
    oc0.wait()
    oc1.wait()


@functools.partial(jax.jit, static_argnames=("A_seg_len",))
def pallas_adaLN_cond__memory_aug_recurrent_mem_tr__dense_activation_gelu__prompt_kernel(
        A_x, A_mem0, A_Wq, A_Wk, A_Wv, A_Wo, A_seg_len, B_x, B_w1, B_b1, B_w2, B_b2, c, w_mod):
    B, S, D = A_x.shape
    H, Dh = A_Wq.shape[1], A_Wq.shape[2]
    M = A_mem0.shape[1]
    Fd = B_w1.shape[1]
    seg = int(A_seg_len)
    assert B == 1 and M == 8 and seg == 32 and Dh == 128
    HD = H * Dh
    anyspec = pl.BlockSpec(memory_space=pl.ANY)
    vm = pl.BlockSpec(memory_space=pltpu.VMEM)
    out = pl.pallas_call(
        functools.partial(_kernel, S=S, D=D, H=H, Dh=Dh, Fd=Fd, M=M, seg=seg),
        out_shape=jax.ShapeDtypeStruct((S, D), BF16),
        in_specs=[anyspec, vm, anyspec, anyspec, anyspec, anyspec, anyspec, vm, anyspec, vm, vm, anyspec],
        out_specs=anyspec,
        scratch_shapes=[
            pltpu.VMEM((S, D), BF16),
            pltpu.VMEM((D // 2, 3 * HD), U32),
            pltpu.VMEM((HD // 2, D), U32),
            pltpu.VMEM((D // 2, Fd), U32),
            pltpu.VMEM((Fd // 2, D), U32),
            pltpu.VMEM((D // 2, 6 * D), U32),
            pltpu.VMEM((7, D, 8, Dh), BF16),
            pltpu.VMEM((64, HD), F32),
            pltpu.VMEM((S, D), F32),
            pltpu.VMEM((S, D), BF16),
            pltpu.SemaphoreType.DMA((7,)),
            pltpu.SemaphoreType.DMA((3 * H // 8,)),
            pltpu.SemaphoreType.DMA((2,)),
        ],
        compiler_params=pltpu.CompilerParams(vmem_limit_bytes=120 * 1024 * 1024, flags={'XLA_TPU_FORCE_LP_LLO_SCHEDULER': True}),
    )(A_x.reshape(S, D), A_mem0.reshape(M, D), A_Wq, A_Wk, A_Wv, A_Wo.reshape(HD, D), B_w1, B_b1,
      B_w2, B_b2, c, w_mod)
    return out.reshape(B, S, D)
```
